```python
import os as _os
_os.environ.setdefault("JAX_PLATFORMS", "cpu")
import jax
import jax.numpy as jnp

def _softmax(x, axis=-1):
    return jax.nn.softmax(x, axis=axis)
def _gelu(x):
    return jax.nn.gelu(x, approximate=True)
def _silu(x):
    return jax.nn.silu(x)
def _sigmoid(x):
    return jax.nn.sigmoid(x)
def _layernorm(x, axis=-1, eps=1e-5):
    m = jnp.mean(x, axis=axis, keepdims=True)
    v = jnp.var(x, axis=axis, keepdims=True)
    return (x - m) / jnp.sqrt(v + eps)
def _scatter_add(tgt, idx, src, axis=0):
    return tgt.at[idx].add(src)
def _segment_sum(src, seg, n):
    return jax.ops.segment_sum(src, seg, n)
class _Rng:
    def __init__(self, key):
        self._k = key
    def _next(self):
        self._k, sub = jax.random.split(self._k)
        return sub
    def normal(self, shape):
        return jax.random.normal(self._next(), shape, dtype=jnp.bfloat16)
    def randint(self, lo, hi, shape):
        return jax.random.randint(self._next(), shape, lo, hi, dtype=jnp.int32)
    def uniform(self, shape, lo=0.0, hi=1.0):
        return jax.random.uniform(self._next(), shape, jnp.bfloat16, lo, hi)
    def permutation(self, n):
        return jax.random.permutation(self._next(), n)


kernel_name = 'gated_mix__mha_block__mixer_s_mlp__prompt'

def setup_inputs():
    _rng = _Rng(jax.random.key(int.from_bytes(__import__("os").urandom(4), "little")))
    _w = (lambda a: (lambda t: t.astype(jnp.bfloat16) if jnp.issubdtype(t.dtype, jnp.floating) else t)(jnp.asarray(a)))
    def _A_setup():
        B, S, D, H = 1, 2048, 512, 32
        return {
            "x": _w((lambda *s: _rng.normal(s) * 0.05)(B, S, D)),
            "wqkv": _w((lambda *s: _rng.normal(s) * 0.8)(D, 3 * D)),
            "wo": _w((lambda *s: _rng.normal(s) * 0.05)(D, D)),
        }
    _A_in = _A_setup()

    def _B_setup():
        B, S, D, F = 1, 2048, 512, 1792
        return {
            "x":  _w((lambda *s: _rng.normal(s) * 0.05)(B, S, D)),
            "w1": _w((lambda *s: _rng.normal(s) * 0.2)(D, D) * (D ** -0.5)),
            "w2": _w((lambda *s: _rng.normal(s) * 0.2)(D, D) * (D ** -0.5)),
            "w3": _w((lambda *s: _rng.normal(s) * 0.2)(D, F) * (D ** -0.5)),
            "w4": _w((lambda *s: _rng.normal(s) * 0.2)(F, D) * (F ** -0.5)),
        }
    _B_in = _B_setup()

    return {
        "A_x": _A_in["x"],
        "A_wqkv": _A_in["wqkv"],
        "A_wo": _A_in["wo"],
        "B_x": _B_in["x"],
        "B_w1": _B_in["w1"],
        "B_w2": _B_in["w2"],
        "B_w3": _B_in["w3"],
        "B_w4": _B_in["w4"],
        "gate_w": _w((lambda *s: _rng.normal(s) * 0.05)(512) * 16.0),
    }

def reference(A_x, A_wqkv, A_wo, B_x, B_w1, B_w2, B_w3, B_w4, gate_w):
    def _A_ref(x, wqkv, wo):
        B, S, D = x.shape
        H = 32
        Dh = D // H
        qkv = (lambda x, *d: x.transpose(*d))((x @ wqkv).reshape(B, S, 3, H, Dh), 2, 0, 3, 1, 4)
        q, k, v = qkv[0], qkv[1], qkv[2]
        scores = jnp.einsum("bhqd,bhkd->bhqk", q, k) * (Dh ** -0.5)
        p = _softmax(scores, axis=-1)
        o = jnp.einsum("bhqk,bhkd->bhqd", p, v)
        return (lambda x, *d: x.transpose(*d))(o, 0, 2, 1, 3).reshape(B, S, D) @ wo

    def _B_ref(x, w1, w2, w3, w4):
        B, S, D = x.shape
        h = _gelu(_layernorm(x, axis=-1) @ w1)
        c = D // 4
        g0 = jnp.pad(h[:, :, 0*c:1*c], ((0, 0), (1, 0), (0, 0)))[:, :S, :]
        g1 = jnp.pad(h[:, :, 1*c:2*c], ((0, 0), (0, 1), (0, 0)))[:, 1:, :]
        g2 = jnp.pad(h[:, :, 2*c:3*c], ((0, 0), (2, 0), (0, 0)))[:, :S, :]
        g3 = jnp.pad(h[:, :, 3*c:   ], ((0, 0), (0, 2), (0, 0)))[:, 2:, :]
        hs = jnp.concatenate([g0, g1, g2, g3], axis=-1) @ w2
        x1 = x + hs
        h2 = _gelu(_layernorm(x1, axis=-1) @ w3) @ w4
        return x1 + h2

    x = A_x
    g = _sigmoid((x * gate_w).sum(-1, keepdims=True))
    a = _A_ref(x, A_wqkv, A_wo)
    b = _B_ref(x, B_w1, B_w2, B_w3, B_w4)
    return g * a + (1 - g) * b
```

```python
import jax
import jax.numpy as jnp
import jax.experimental.pallas as pl
import jax.experimental.pallas.tpu as pltpu

S, D, H, DH, F = 2048, 512, 32, 16, 1792
G = D // 128
HG = H // G
RB = 512
NB = S // RB
KC = 128
NC = S // KC
PAD = 8
VROWS = list(range(0, KC, 16)) + [S - 16]
VK = 16 * len(VROWS)
CUTS = [KC] + list(range(288, 1697, KC)) + [1776, 1856, 1936, S - 16]
OUT_CUTS = (0, 512, 1024, 1536, 1792, 1920, 2048)
QSCALE = DH ** -0.5 * 1.4426950408889634
L_LO, L_HI = 2.0 ** -30, 2.0 ** 100
F32_MAX = 3.0e38

f32, bf16 = jnp.float32, jnp.bfloat16


def _dot(a, b):
    return jnp.dot(a, b, preferred_element_type=f32)


def _flip(x):
    return jnp.concatenate(
        [x[c + r:c + r + 16] for c in range(0, x.shape[0], KC) for r in range(KC - 16, -1, -16)],
        axis=0)


def _layernorm(x):
    m = jnp.mean(x, axis=-1, keepdims=True)
    d = x - m
    v = jnp.mean(d * d, axis=-1, keepdims=True)
    return d * jax.lax.rsqrt(v + 1e-5)


def _gelu(x):
    c0 = 0.7978845608028654
    t = jnp.tanh(x * (c0 + (c0 * 0.044715) * (x * x)))
    hx = 0.5 * x
    return hx + hx * t


def _values_plan(units):
    ns = len(CUTS) - 1
    ready = []
    for u in range(units):
        ready.append(((u + 1) * ns - 0.5, u, 0))
        for c in range(1, NC):
            n = min(n for n in range(ns) if CUTS[n + 1] >= min((c + 1) * KC, CUTS[-1]))
            ready.append((u * ns + n + 1, u, c))
    follow, at = [[] for _ in range(units * ns + 1)], 0
    for m, u, c in sorted(ready):
        at = min(max(at, int(m)), units * ns)
        follow[at].append((u, c))
        at += 1
    return follow


def _kernel(x_hbm, wqkv_hbm, wo_hbm, w1_hbm, w2_hbm, w3_hbm, w4_hbm, gw_ref,
            out_hbm,
            x_s, wqkv, wo, w1, w2, w3, w4,
            k_s, qt_s, vt_s, ot_s, h_s, b_s, o_s, g_s, bad_s, kb_s, in_sem, out_sem):

    def rows(i):
        return pl.ds(pl.multiple_of(i * RB, RB), RB)

    def copy(n, src, dst):
        return pltpu.make_async_copy(src, dst, in_sem.at[n])

    x_cp = [copy(i, x_hbm.at[i * RB:(i + 1) * RB], x_s.at[i * RB:(i + 1) * RB])
            for i in range(NB)]
    w_cp = [copy(NB + j, wqkv_hbm.at[:, j * D:(j + 1) * D], wqkv.at[:, j * D:(j + 1) * D])
            for j in range(3)]
    w1_cp = copy(NB + 3, w1_hbm, w1)
    late_cp = [copy(NB + 4 + n, s, d) for n, (s, d) in enumerate(
        [(w2_hbm, w2), (w3_hbm, w3), (w4_hbm, w4), (wo_hbm, wo)])]

    x_cp[0].start()
    for c in w_cp:
        c.start()
    h_s[0:PAD, :] = jnp.zeros((PAD, D), f32)
    h_s[PAD + S:PAD + S + PAD, :] = jnp.zeros((PAD, D), f32)
    bad_s[...] = jnp.zeros((DH, RB), f32)
    x_cp[0].wait()
    w_cp[0].wait()
    w1_cp.start()

    def proj_block(i, first):
        x = x_s[rows(i), :]
        q = _dot(x, wqkv[:, 0:D]) * QSCALE
        qt_s[i] = q.T.reshape(G, HG, DH, RB)
        if first:
            for c in x_cp[1:]:
                c.start()
            w_cp[1].wait()
            w_cp[2].wait()
        v = _dot(x, wqkv[:, 2 * D:3 * D])
        vt_s[i] = v.astype(bf16).T.reshape(H, DH, RB)
        xf = x.astype(f32)
        z = jnp.sum(xf * gw_ref[...].astype(f32).reshape(1, D), axis=-1, keepdims=True)
        g_s[rows(i), :] = jnp.broadcast_to(jax.nn.sigmoid(z), (RB, 128))
        y = _layernorm(xf).astype(bf16)
        if first:
            w1_cp.wait()
        h_s[pl.ds(pl.multiple_of(i * RB + PAD, 8), RB), :] = _gelu(_dot(y, w1[...]))
        k = _flip(_dot(x, wqkv[:, D:2 * D])).astype(bf16)
        for g in range(G):
            k_s[g, rows(i), :] = k[:, g * 128:(g + 1) * 128]

    def proj_step(i, carry):
        proj_block(i + 1, False)
        return carry

    proj_block(0, True)
    for c in x_cp[1:]:
        c.wait()
    for c in late_cp:
        c.start()
    jax.lax.fori_loop(0, NB - 1, proj_step, 0)
    for c in late_cp:
        c.wait()

    def gate(r):
        return jnp.concatenate([g_s[r, :]] * (D // 128), axis=1)

    def spread_keys(h):
        k = jnp.concatenate([k_s[h // HG, r:r + 16, :].astype(f32) for r in VROWS], axis=0)
        k = pltpu.roll(k, (HG - h % HG) % HG * DH, 1)
        for t in range(VK // 8):
            for d in range(DH):
                kb_s[h, t, d] = jnp.broadcast_to(k[8 * t:8 * t + 8, d:d + 1], (8, 128))

    def mlp_block(i, carry):
        heads = iter(range(HG))
        hh = h_s[pl.ds(pl.multiple_of(i * RB, 8), RB + 2 * PAD), :]
        parts = [hh[PAD - sh:PAD - sh + RB, j * 128:(j + 1) * 128].astype(bf16)
                 for j, sh in enumerate((1, -1, 2, -2))]
        x1 = x_s[rows(i), :].astype(f32) + _dot(jnp.concatenate(parts, axis=-1), w2[...])
        y = _layernorm(x1).astype(bf16)
        spread_keys(i * HG + next(heads))
        u = []
        for a in range(0, F, 512):
            u.append(_gelu(_dot(y, w3[:, a:min(a + 512, F)])))
            spread_keys(i * HG + next(heads))
        u = jnp.concatenate(u, axis=1).astype(bf16)
        for a in range(0, F, 256):
            x1 = x1 + _dot(u[:, a:a + 256], w4[a:a + 256, :])
            if a < 3 * 256:
                spread_keys(i * HG + next(heads))
        b_s[rows(i), :] = (1.0 - gate(rows(i))) * x1
        return carry

    jax.lax.fori_loop(0, NB, mlp_block, 0)

    def masked_q(qb, h):
        row = jax.lax.broadcasted_iota(jnp.int32, (128, RB), 0) // DH
        return jnp.where(row == h % HG, qt_s[qb, h // HG].reshape(128, RB), 0.0).astype(bf16)

    def fast_step(step, carry):
        units = [(2 * step + j, qb) for j in range(2) for qb in range(NB)]
        ns, tiles = len(CUTS) - 1, range(0, RB, 128)
        follow = _values_plan(len(units))
        vitems = [(r0, y) for r0 in range(len(VROWS)) for y in range(len(tiles))]
        w, l, acc, p, pv = {}, {}, {}, {}, {}
        left = [NC] * len(units)
        bad = [bad_s[...]]

        def vector_scores(u, t, y):
            h, qb = units[u]
            s = [None, None]
            for d in range(DH):
                qd = jnp.broadcast_to(
                    qt_s[qb, h // HG, h % HG, d:d + 1, tiles[y]:tiles[y] + 128], (8, 128))
                for a in range(2):
                    prod = kb_s[h, 2 * t + a, d] * qd
                    s[a] = prod if d == 0 else s[a] + prod
            e = [jnp.exp2(x) for x in s]
            l[u][y] = l[u][y] + (e[0] + e[1])
            pv[u, VROWS[t], y] = jnp.concatenate(e, axis=0)

        def scores(u, n):
            (h, qb), lo, hi = units[u], CUTS[n], CUTS[n + 1]
            if n == 0:
                w[u] = masked_q(qb, h)
                l[u] = [jnp.zeros((8, 128), f32)] * len(tiles)
                acc[u] = jnp.zeros((DH, RB), f32)
            e = jnp.exp2(_dot(k_s[h // HG, lo:hi, :], w[u]))
            es = e.reshape((hi - lo) // 8, 8, RB).sum(0)
            l[u] = [x + es[:, y:y + 128] for x, y in zip(l[u], tiles)]
            for r in range(lo, hi, 16):
                p[u, r] = e[r - lo:r - lo + 16]
            nv = len(vitems)
            for t, y in vitems[n * nv // (ns - 1):(n + 1) * nv // (ns - 1)]:
                vector_scores(u, t, y)

        def values(u, c):
            h, qb = units[u]
            pp = [jnp.concatenate([pv.pop((u, r, y)) for y in range(len(tiles))], axis=1)
                  if r in VROWS else p.pop((u, r))
                  for r in range((c + 1) * KC - 16, c * KC - 1, -16)]
            lane = c % (RB // KC) * KC
            acc[u] = acc[u] + _dot(vt_s[c // (RB // KC), h, :, lane:lane + KC],
                                   jnp.concatenate(pp, axis=0).astype(bf16))
            left[u] -= 1
            if not left[u]:
                ls = jnp.sum(jnp.concatenate(l[u], axis=1), axis=0, keepdims=True)
                ok = (ls >= L_LO) & (ls <= L_HI) & (jnp.abs(acc[u]) <= F32_MAX)
                bad[0] = jnp.where(ok, bad[0], 1.0)
                ot_s[qb, h] = (acc[u] / ls).astype(bf16)

        for u in range(len(units)):
            for n in range(ns):
                scores(u, n)
                for item in follow[u * ns + n]:
                    values(*item)
        for item in follow[-1]:
            values(*item)
        bad_s[...] = bad[0]
        return carry

    def safe_step(i, carry):
        qb, h = i // H, i % H
        w = masked_q(qb, h)

        def scores(c):
            return _dot(k_s[h // HG, rows(c), :], w)

        m = jax.lax.fori_loop(
            0, NB, lambda c, m: jnp.maximum(m, jnp.max(scores(c), axis=0, keepdims=True)),
            jnp.full((1, RB), -jnp.inf, f32))

        def accumulate(c, state):
            l, acc = state
            e = jnp.exp2(scores(c) - m)
            return (l + jnp.sum(e, axis=0, keepdims=True),
                    acc + _dot(vt_s[c, h], _flip(e).astype(bf16)))

        l, acc = jax.lax.fori_loop(
            0, NB, accumulate, (jnp.zeros((1, RB), f32), jnp.zeros((DH, RB), f32)))
        ot_s[qb, h] = (acc / l).astype(bf16)
        return carry

    jax.lax.fori_loop(0, H // 2, fast_step, 0)

    @pl.when(jnp.max(bad_s[...]) > 0.0)
    def _():
        jax.lax.fori_loop(0, NB * H, safe_step, 0)

    out_cp = []
    for n, (lo, hi) in enumerate(zip(OUT_CUTS[:-1], OUT_CUTS[1:])):
        if lo % RB == 0:
            o = ot_s[lo // RB].reshape(D, RB).T
        a = _dot(o[lo % RB:lo % RB + hi - lo], wo[...])
        o_s[lo:hi, :] = (gate(slice(lo, hi)) * a + b_s[lo:hi, :]).astype(bf16)
        out_cp.append(pltpu.make_async_copy(o_s.at[lo:hi], out_hbm.at[lo:hi], out_sem.at[n]))
        out_cp[-1].start()
    for c in out_cp:
        c.wait()


@jax.jit
def pallas_gated_mix__mha_block__mixer_s_mlp__prompt_kernel(
    A_x: jax.Array,
    A_wqkv: jax.Array,
    A_wo: jax.Array,
    B_x: jax.Array,
    B_w1: jax.Array,
    B_w2: jax.Array,
    B_w3: jax.Array,
    B_w4: jax.Array,
    gate_w: jax.Array,
):
    del B_x
    any_spec = pl.BlockSpec(memory_space=pl.ANY)
    out = pl.pallas_call(
        _kernel,
        out_shape=jax.ShapeDtypeStruct((S, D), bf16),
        in_specs=[any_spec] * 7 + [pl.BlockSpec(memory_space=pltpu.VMEM)],
        out_specs=any_spec,
        scratch_shapes=[
            pltpu.VMEM((S, D), bf16),
            pltpu.VMEM((D, 3 * D), bf16),
            pltpu.VMEM((D, D), bf16),
            pltpu.VMEM((D, D), bf16),
            pltpu.VMEM((D, D), bf16),
            pltpu.VMEM((D, F), bf16),
            pltpu.VMEM((F, D), bf16),
            pltpu.VMEM((G, S, 128), bf16),
            pltpu.VMEM((NB, G, HG, DH, RB), f32),
            pltpu.VMEM((NB, H, DH, RB), bf16),
            pltpu.VMEM((NB, H, DH, RB), bf16),
            pltpu.VMEM((S + 2 * PAD, D), f32),
            pltpu.VMEM((S, D), f32),
            pltpu.VMEM((S, D), bf16),
            pltpu.VMEM((S, 128), f32),
            pltpu.VMEM((DH, RB), f32),
            pltpu.VMEM((H, VK // 8, DH, 8, 128), f32),
            pltpu.SemaphoreType.DMA((NB + 8,)),
            pltpu.SemaphoreType.DMA((len(OUT_CUTS) - 1,)),
        ],
        compiler_params=pltpu.CompilerParams(vmem_limit_bytes=100 * 1024 * 1024),
    )(A_x.reshape(S, D), A_wqkv, A_wo, B_w1, B_w2, B_w3, B_w4, gate_w)
    return out.reshape(1, S, D)
```
